```python
import os as _os
_os.environ.setdefault("JAX_PLATFORMS", "cpu")
import jax
import jax.numpy as jnp

def _softmax(x, axis=-1):
    return jax.nn.softmax(x, axis=axis)
def _gelu(x):
    return jax.nn.gelu(x, approximate=True)
def _silu(x):
    return jax.nn.silu(x)
def _sigmoid(x):
    return jax.nn.sigmoid(x)
def _layernorm(x, axis=-1, eps=1e-5):
    m = jnp.mean(x, axis=axis, keepdims=True)
    v = jnp.var(x, axis=axis, keepdims=True)
    return (x - m) / jnp.sqrt(v + eps)
def _scatter_add(tgt, idx, src, axis=0):
    return tgt.at[idx].add(src)
def _segment_sum(src, seg, n):
    return jax.ops.segment_sum(src, seg, n)
class _Rng:
    def __init__(self, key):
        self._k = key
    def _next(self):
        self._k, sub = jax.random.split(self._k)
        return sub
    def normal(self, shape):
        return jax.random.normal(self._next(), shape, dtype=jnp.bfloat16)
    def randint(self, lo, hi, shape):
        return jax.random.randint(self._next(), shape, lo, hi, dtype=jnp.int32)
    def uniform(self, shape, lo=0.0, hi=1.0):
        return jax.random.uniform(self._next(), shape, jnp.bfloat16, lo, hi)
    def permutation(self, n):
        return jax.random.permutation(self._next(), n)


kernel_name = 'standalone__channel_attn_cbam__vision'

def setup_inputs():
    _rng = _Rng(jax.random.key(int.from_bytes(__import__("os").urandom(4), "little")))
    _w = (lambda a: (lambda t: t.astype(jnp.bfloat16) if jnp.issubdtype(t.dtype, jnp.floating) else t)(jnp.asarray(a)))
    H = W = 384
    C = 192
    r = max(C // 4, 1)
    return {
        "x": _w((lambda *s: _rng.normal(s) * 0.2)(1, H, W, C) + (lambda *s: _rng.normal(s) * 0.2)(1, 1, 1, C) * 2.0),
        "w1": _w((lambda *s: _rng.normal(s) * 0.2)(C, r)),
        "w2": _w((lambda *s: _rng.normal(s) * 0.2)(r, C)),
    }

def reference(x, w1, w2):
    B, H, W, C = x.shape
    xf = x.reshape(B, H * W, C)
    gap = jnp.mean(xf, 1)
    gmp = jnp.amax(xf, 1)
    h_a = gap @ w1
    h_a = h_a * (lambda x, dt: x.astype(dt))(h_a > 0, h_a.dtype)
    h_m = gmp @ w1
    h_m = h_m * (lambda x, dt: x.astype(dt))(h_m > 0, h_m.dtype)
    scale = _sigmoid(h_a @ w2 + h_m @ w2)
    return x * scale[:, None, None, :]
```

```python
import functools
import jax
import jax.numpy as jnp
from jax import lax
from jax.experimental import pallas as pl
from jax.experimental.pallas import tpu as pltpu

H, W, C, R = 384, 384, 192, 48
NSEG, NJ = 54, 64
NCG = C // 8
NPH = 9


def to_view(x):
    t = x.reshape(H, W, C).transpose(0, 2, 1).reshape(H, NCG, 8, 3, 128).transpose(0, 1, 3, 2, 4)
    t = t.reshape(NSEG * NJ, 8, 8, 128).transpose(0, 2, 1, 3)
    return t.reshape(NSEG, NJ, 8, 1024)


def from_view(y):
    t = y.reshape(NSEG * NJ, 8, 8, 128).transpose(0, 2, 1, 3)
    t = t.reshape(H, NCG, 3, 8, 128).transpose(0, 1, 3, 2, 4).reshape(H, C, W)
    return t.transpose(0, 2, 1).reshape(1, H, W, C)


def _bf(v):
    return v.astype(jnp.bfloat16).astype(jnp.float32)


def make(name='cbam', D=8, nsplit=2, a0=4, WA=6, do_compute=True, mlp='vpu'):
    RA = 9
    NSTEP = (NSEG // RA) * NJ
    RING = D + 1
    lw = 1024 // nsplit
    WG = NSEG // WA

    def kernel(x_hbm, w1t_hbm, w2_hbm, o_hbm, buf, w1t_v, w2_v, acc_s, acc_m, w1d, w2d, tab,
               sem_in, sem_w, sem_out):
        def issue(i):
            g = i // NJ
            j = i % NJ
            sem = sem_in.at[i % RING]
            for h in range(nsplit):
                ls = pl.ds(h * lw, lw)
                pltpu.make_async_copy(x_hbm.at[pl.ds(g * RA, a0), j, :, ls],
                                      buf.at[pl.ds(g * RA, a0), j, :, ls], sem).start(priority=0)
                pltpu.make_async_copy(x_hbm.at[pl.ds(g * RA + a0, RA - a0), j, :, ls],
                                      buf.at[pl.ds(g * RA + a0, RA - a0), j, :, ls], sem).start(priority=1)

        def wait(i):
            g = i // NJ
            j = i % NJ
            pltpu.make_async_copy(x_hbm.at[pl.ds(g * RA, RA), j], buf.at[pl.ds(g * RA, RA), j],
                                  sem_in.at[i % RING]).wait()

        cw1 = pltpu.make_async_copy(w1t_hbm, w1t_v, sem_w.at[0])
        cw2 = pltpu.make_async_copy(w2_hbm, w2_v, sem_w.at[1])
        for i in range(D):
            issue(i)
        cw1.start()
        cw2.start()
        acc_s[...] = jnp.zeros(acc_s.shape, jnp.float32)
        acc_m[...] = jnp.full(acc_m.shape, -jnp.inf, jnp.float32)
        cw1.wait()
        cw2.wait()
        def dup(ref):
            w = ref[...].astype(jnp.float32)
            z = jnp.zeros((16, C), jnp.float32)
            return jnp.concatenate([w, z, w, z], axis=0).T
        w1d[...] = dup(w1t_v)
        w2d[...] = dup(w2_v)

        def reduce_step(i):
            g = i // NJ
            j = i % NJ
            r = lax.rem(j, NPH)
            tiles = []
            for p in range(NPH):
                a = p - r
                a = jnp.where(a < 0, a + NPH, a)
                v = buf[g * RA + a, j].astype(jnp.float32)
                tiles += [v[:, 128 * k:128 * (k + 1)] for k in range(8)]
            for cg in range(NCG):
                t0, t1, t2 = tiles[3 * cg:3 * cg + 3]
                rows = pl.ds(8 * cg, 8)
                acc_s[rows, :] = acc_s[rows, :] + ((t0 + t1) + t2)
                acc_m[rows, :] = jnp.maximum(acc_m[rows, :], jnp.maximum(jnp.maximum(t0, t1), t2))

        def body1(i, c):
            issue(i + D)
            wait(i)
            if do_compute:
                reduce_step(i)
            return c
        lax.fori_loop(0, NSTEP - D, body1, 0)

        def body2(i, c):
            wait(i)
            if do_compute:
                reduce_step(i)
            return c
        lax.fori_loop(NSTEP - D, NSTEP, body2, 0)

        gap = _bf(jnp.sum(acc_s[...], axis=1, keepdims=True) * (1.0 / (H * W)))
        gmp = jnp.max(acc_m[...], axis=1, keepdims=True)
        lane = lax.broadcasted_iota(jnp.int32, (C, 128), 1)
        pooled = jnp.where(lane < 64, gap, gmp)
        hid = _bf(jnp.sum(w1d[...] * pooled, axis=0, keepdims=True))
        hid = jnp.maximum(hid, 0.0)
        z = jnp.sum(w2d[...] * hid, axis=1, keepdims=True)
        scale = _bf(jax.nn.sigmoid(z))
        scale = jnp.broadcast_to(scale, (C, 128))
        for u in range(3 * NCG):
            cg = u // 3
            tab[u // 8, :, pl.ds(128 * (u % 8), 128)] = scale[8 * cg:8 * cg + 8, :]

        def body3(i, c):
            g = i // NJ
            j = i % NJ
            if do_compute:
                r = lax.rem(g * WA + j, NPH)
                for a in range(WA):
                    p = r + a
                    p = jnp.where(p >= NPH, p - NPH, p)
                    s = g * WA + a
                    buf[s, j] = (buf[s, j].astype(jnp.float32) * tab[p]).astype(jnp.bfloat16)
            pltpu.make_async_copy(buf.at[pl.ds(g * WA, WA), j], o_hbm.at[pl.ds(g * WA, WA), j],
                                  sem_out.at[0]).start()
            return c
        lax.fori_loop(0, WG * NJ, body3, 0)
        pltpu.make_async_copy(buf, o_hbm, sem_out.at[0]).wait()

    @jax.jit
    def f(x, w1, w2):
        out = pl.pallas_call(
            kernel, name=name,
            out_shape=jax.ShapeDtypeStruct((NSEG, NJ, 8, 1024), jnp.bfloat16),
            in_specs=[pl.BlockSpec(memory_space=pl.ANY)] * 3,
            out_specs=pl.BlockSpec(memory_space=pl.ANY),
            scratch_shapes=[
                pltpu.VMEM((NSEG, NJ, 8, 1024), jnp.bfloat16),
                pltpu.VMEM((R, C), jnp.bfloat16),
                pltpu.VMEM((R, C), jnp.bfloat16),
                pltpu.VMEM((C, 128), jnp.float32),
                pltpu.VMEM((C, 128), jnp.float32),
                pltpu.VMEM((C, 128), jnp.float32),
                pltpu.VMEM((C, 128), jnp.float32),
                pltpu.VMEM((NPH, 8, 1024), jnp.float32),
                pltpu.SemaphoreType.DMA((RING,)),
                pltpu.SemaphoreType.DMA((2,)),
                pltpu.SemaphoreType.DMA((1,)),
            ],
            compiler_params=pltpu.CompilerParams(vmem_limit_bytes=100 * 1024 * 1024,
                                                 disable_semaphore_checks=True),
        )(to_view(x), w1.T, w2)
        return from_view(out)
    return f


_impl = make()


@jax.jit
def pallas_standalone__channel_attn_cbam__vision_kernel(x, w1, w2):
    return _impl(x, w1, w2)
```

```python
import functools

import jax
import jax.numpy as jnp
from jax import lax
import jax.experimental.pallas as pl
import jax.experimental.pallas.tpu as pltpu

F32 = jnp.float32
BF16 = jnp.bfloat16

H, W, C, R = 384, 384, 192, 48
NCG = C // 8
WT = W // 128
NPH = NCG * WT // 8
NSEG, NJ = 54, 64
CW = 1024

RA = NPH
RSPLIT = 4
RHI = 2
DEPTH = 12
RING = 16
NREAD = (NSEG // RA) * NJ

WA = 6
RAMP = 2
NWRITE = (NSEG // WA) * NJ


def _to_view(x):
    t = x.reshape(H, W, C).transpose(0, 2, 1)
    t = t.reshape(H, NCG, 8, WT, 128).transpose(0, 1, 3, 2, 4)
    t = t.reshape(NSEG * NJ, 8, 8, 128).transpose(0, 2, 1, 3)
    return t.reshape(NSEG, NJ, 8, CW)


def _from_view(y):
    t = y.reshape(NSEG * NJ, 8, 8, 128).transpose(0, 2, 1, 3)
    t = t.reshape(H, NCG, WT, 8, 128).transpose(0, 1, 3, 2, 4)
    return t.reshape(H, C, W).transpose(0, 2, 1).reshape(1, H, W, C)


def _bf(v):
    return v.astype(BF16).astype(F32)


def _cbam_kernel(x_hbm, w1t_hbm, w2_hbm, o_hbm,
                 buf, w1t_v, w2_v, acc_s, acc_m, w1d, w2d, tab,
                 sem_in, sem_w, sem_out):
    def split(i):
        if isinstance(i, int):
            return (i // NJ) * RA, i % NJ, i % RING
        return lax.shift_right_logical(i, 6) * RA, i & (NJ - 1), i & (RING - 1)

    def issue(i):
        s0, j, slot = split(i)
        lw = CW // RSPLIT
        for h in range(RSPLIT):
            for a, n, prio in ((0, RHI, 0), (RHI, RA - RHI, 1)):
                idx = (pl.ds(s0 + a, n), j, slice(None), pl.ds(h * lw, lw))
                pltpu.make_async_copy(x_hbm.at[idx], buf.at[idx],
                                      sem_in.at[slot]).start(priority=prio)

    def wait(i):
        s0, j, slot = split(i)
        idx = (pl.ds(s0, RA), j)
        pltpu.make_async_copy(x_hbm.at[idx], buf.at[idx], sem_in.at[slot]).wait()

    def pooled(i):
        s0, j, _ = split(i)
        if isinstance(j, int):
            segs = [(p - j) % NPH for p in range(NPH)]
        else:
            r = j - NPH * lax.shift_right_logical(j * 57, 9)
            segs = [jnp.where(p - r < 0, p - r + NPH, p - r) for p in range(NPH)]
        tiles = []
        for a in segs:
            v = buf[s0 + a, j].astype(F32)
            tiles += [v[:, 128 * k:128 * (k + 1)] for k in range(8)]
        out = []
        for cg in range(NCG):
            rows = pl.ds(8 * cg, 8)
            ts = tiles[WT * cg:WT * (cg + 1)]
            out.append((acc_s[rows, :] + functools.reduce(jnp.add, ts),
                        jnp.maximum(acc_m[rows, :], functools.reduce(jnp.maximum, ts))))
        return out

    def accumulate(i):
        for cg, (s, m) in enumerate(pooled(i)):
            acc_s[pl.ds(8 * cg, 8), :] = s
            acc_m[pl.ds(8 * cg, 8), :] = m

    cw1 = pltpu.make_async_copy(w1t_hbm, w1t_v, sem_w.at[0])
    cw2 = pltpu.make_async_copy(w2_hbm, w2_v, sem_w.at[1])
    issue(0)
    cw1.start()
    cw2.start()
    for i in range(1, DEPTH):
        issue(i)
    acc_s[...] = jnp.zeros(acc_s.shape, F32)
    acc_m[...] = jnp.full(acc_m.shape, -jnp.inf, F32)
    cw1.wait()
    cw2.wait()

    def dup(ref):
        w = ref[...].astype(F32)
        z = jnp.zeros((64 - R, C), F32)
        return jnp.concatenate([w, z, w, z], axis=0).T

    w1d[...] = dup(w1t_v)
    w2d[...] = dup(w2_v) * 0.5

    def read_body(i, c):
        issue(i + DEPTH)
        wait(i)
        accumulate(i)
        return c

    def drain_body(i, c):
        wait(i)
        accumulate(i)
        return c

    lax.fori_loop(0, NREAD - DEPTH, read_body, 0)
    lax.fori_loop(NREAD - DEPTH, NREAD - 1, drain_body, 0)
    wait(NREAD - 1)

    avg_lane = lax.broadcasted_iota(jnp.int32, (8, 128), 1) < 64
    terms = []
    for cg, (s, m) in enumerate(pooled(NREAD - 1)):
        gap = _bf(jnp.sum(s, axis=1, keepdims=True) * (1.0 / (H * W)))
        gmp = jnp.max(m, axis=1, keepdims=True)
        terms.append(w1d[pl.ds(8 * cg, 8), :] * jnp.where(avg_lane, gap, gmp))
    hid = _bf(jnp.sum(functools.reduce(jnp.add, terms), axis=0, keepdims=True))
    hid = jnp.maximum(hid, 0.0)
    scale = []
    for cg in range(NCG):
        prod = w2d[pl.ds(8 * cg, 8), :] * hid
        za = jnp.sum(jnp.where(avg_lane, prod, 0.0), axis=1, keepdims=True)
        zm = jnp.sum(jnp.where(avg_lane, 0.0, prod), axis=1, keepdims=True)
        gate = _bf(0.5 * jnp.tanh(_bf(_bf(za) + _bf(zm))) + 0.5)
        scale.append(jnp.broadcast_to(gate, (8, 128)))

    def put(idx):
        pltpu.make_async_copy(buf.at[idx], o_hbm.at[idx], sem_out.at[0]).start()

    for j in range(RAMP):
        for a in range(WA):
            p = (a + j) % NPH
            row = jnp.concatenate([scale[(8 * p + k) // WT] for k in range(8)], axis=1)
            buf[a, j] = (buf[a, j].astype(F32) * row).astype(BF16)
            if j == 0:
                put((a, j))
        if j > 0:
            put((pl.ds(0, WA), j))

    for u in range(NCG * WT):
        tab[u // 8, :, pl.ds(128 * (u % 8), 128)] = scale[u // WT]

    def write_body(i, r):
        s0 = lax.shift_right_logical(i, 6) * WA
        j = i & (NJ - 1)
        for a in range(WA):
            p = jnp.where(r + a >= NPH, r + a - NPH, r + a)
            buf[s0 + a, j] = (buf[s0 + a, j].astype(F32) * tab[p]).astype(BF16)
        put((pl.ds(s0, WA), j))
        r = r + jnp.where(j == NJ - 1, (WA - (NJ - 1)) % NPH, 1)
        return jnp.where(r >= NPH, r - NPH, r)

    lax.fori_loop(RAMP, NWRITE, write_body, jnp.int32(RAMP))
    pltpu.make_async_copy(buf, o_hbm, sem_out.at[0]).wait()


@jax.jit
def pallas_standalone__channel_attn_cbam__vision_kernel(
    x: jax.Array,
    w1: jax.Array,
    w2: jax.Array,
):
    assert x.shape == (1, H, W, C) and w1.shape == (C, R) and w2.shape == (R, C)
    out = pl.pallas_call(
        _cbam_kernel,
        out_shape=jax.ShapeDtypeStruct((NSEG, NJ, 8, CW), BF16),
        in_specs=[pl.BlockSpec(memory_space=pl.ANY)] * 3,
        out_specs=pl.BlockSpec(memory_space=pl.ANY),
        scratch_shapes=[
            pltpu.VMEM((NSEG, NJ, 8, CW), BF16),
            pltpu.VMEM((R, C), BF16),
            pltpu.VMEM((R, C), BF16),
            pltpu.VMEM((C, 128), F32),
            pltpu.VMEM((C, 128), F32),
            pltpu.VMEM((C, 128), F32),
            pltpu.VMEM((C, 128), F32),
            pltpu.VMEM((NPH, 8, CW), F32),
            pltpu.SemaphoreType.DMA((RING,)),
            pltpu.SemaphoreType.DMA((2,)),
            pltpu.SemaphoreType.DMA((1,)),
        ],
        compiler_params=pltpu.CompilerParams(
            vmem_limit_bytes=64 * 1024 * 1024,
            disable_semaphore_checks=True,
            disable_bounds_checks=True,
        ),
    )(_to_view(x), w1.T, w2)
    return _from_view(out)
```

```python
import functools

import jax
import jax.numpy as jnp
from jax import lax
import jax.experimental.pallas as pl
import jax.experimental.pallas.tpu as pltpu

F32 = jnp.float32
BF16 = jnp.bfloat16

H, W, C, R = 384, 384, 192, 48
NCG = C // 8
WT = W // 128
NPH = NCG * WT // 8
NSEG, NJ = 54, 64
CW = 1024

RA = 2 * NPH
RHI = 2
AHEAD = (3, 5)
RING = 8
NREAD = (NSEG // RA) * NJ

WA = 6
RAMP = 2
WLAG = 8
WRING = 16
NWRITE = (NSEG // WA) * NJ


def _to_view(x):
    t = x.reshape(H, W, C).transpose(0, 2, 1)
    t = t.reshape(H, NCG, 8, WT, 128).transpose(0, 1, 3, 2, 4)
    t = t.reshape(NSEG * NJ, 8, 8, 128).transpose(0, 2, 1, 3)
    return t.reshape(NSEG, NJ, 8, CW)


def _from_view(y):
    t = y.reshape(NSEG * NJ, 8, 8, 128).transpose(0, 2, 1, 3)
    t = t.reshape(H, NCG, WT, 8, 128).transpose(0, 1, 3, 2, 4)
    return t.reshape(H, C, W).transpose(0, 2, 1).reshape(1, H, W, C)


def _bf(v):
    return v.astype(BF16).astype(F32)


def _cbam_kernel(x_hbm, w1t_hbm, w2_hbm, o_hbm,
                 buf, w1t_v, w2_v, acc_s, acc_m, w1d, w2d, tab,
                 sem_in, sem_w, sem_out):
    def split(i):
        if isinstance(i, int):
            return (i // NJ) * RA, i % NJ, i % RING
        return lax.shift_right_logical(i, 6) * RA, i & (NJ - 1), i & (RING - 1)

    def fetch(steps):
        for k in range(8):
            for prio, i in enumerate(steps):
                if i is None:
                    continue
                s0, j, slot = split(i)
                a, n = ((RA - RHI, RHI), (0, RA - RHI))[prio]
                idx = (pl.ds(s0 + a, n), j, slice(None), pl.ds(128 * k, 128))
                pltpu.make_async_copy(x_hbm.at[idx], buf.at[idx],
                                      sem_in.at[slot]).start(priority=prio)

    def wait(i):
        s0, j, slot = split(i)
        idx = (pl.ds(s0, RA), j)
        pltpu.make_async_copy(x_hbm.at[idx], buf.at[idx], sem_in.at[slot]).wait()

    def pooled(i):
        s0, j, _ = split(i)
        if isinstance(j, int):
            segs = [(p - j) % NPH for p in range(NPH)]
        else:
            r = j - NPH * lax.shift_right_logical(j * 57, 9)
            segs = [jnp.where(p - r < 0, p - r + NPH, p - r) for p in range(NPH)]
        tiles = [[] for _ in range(NCG)]
        for b in range(0, RA, NPH):
            for p, a in enumerate(segs):
                v = buf[s0 + b + a, j].astype(F32)
                for k in range(8):
                    tiles[(8 * p + k) // WT].append(v[:, 128 * k:128 * (k + 1)])
        out = []
        for cg, ts in enumerate(tiles):
            rows = pl.ds(8 * cg, 8)
            out.append((acc_s[rows, :] + functools.reduce(jnp.add, ts),
                        jnp.maximum(acc_m[rows, :], functools.reduce(jnp.maximum, ts))))
        return out

    def accumulate(i):
        for cg, (s, m) in enumerate(pooled(i)):
            acc_s[pl.ds(8 * cg, 8), :] = s
            acc_m[pl.ds(8 * cg, 8), :] = m

    cw1 = pltpu.make_async_copy(w1t_hbm, w1t_v, sem_w.at[0])
    cw2 = pltpu.make_async_copy(w2_hbm, w2_v, sem_w.at[1])
    fetch((0, 0))
    cw1.start()
    cw2.start()
    for i in range(1, AHEAD[1] - 1):
        fetch((i if i < AHEAD[0] else None, i))
    acc_s[...] = jnp.zeros(acc_s.shape, F32)
    acc_m[...] = jnp.full(acc_m.shape, -jnp.inf, F32)
    cw1.wait()
    cw2.wait()

    def dup(ref):
        w = ref[...].astype(F32)
        z = jnp.zeros((64 - R, C), F32)
        return jnp.concatenate([w, z, w, z], axis=0).T

    w1d[...] = dup(w1t_v)
    w2d[...] = dup(w2_v) * 0.5

    fetch((None, AHEAD[1] - 1))

    def read_body(lo, i, c):
        fetch([i + d if lo + d < NREAD else None for d in AHEAD])
        wait(i)
        accumulate(i)
        return c

    cuts = (0, NREAD - AHEAD[1], NREAD - AHEAD[0], NREAD - 1)
    for lo, hi in zip(cuts[:-1], cuts[1:]):
        lax.fori_loop(lo, hi, functools.partial(read_body, lo), 0)
    wait(NREAD - 1)

    avg_lane = lax.broadcasted_iota(jnp.int32, (8, 128), 1) < 64
    terms = []
    for cg, (s, m) in enumerate(pooled(NREAD - 1)):
        gap = _bf(jnp.sum(s, axis=1, keepdims=True) * (1.0 / (H * W)))
        gmp = jnp.max(m, axis=1, keepdims=True)
        terms.append(w1d[pl.ds(8 * cg, 8), :] * jnp.where(avg_lane, gap, gmp))
    hid = _bf(jnp.sum(functools.reduce(jnp.add, terms), axis=0, keepdims=True))
    hid = jnp.maximum(hid, 0.0)
    scale = []
    for cg in range(NCG):
        prod = w2d[pl.ds(8 * cg, 8), :] * hid
        za = jnp.sum(jnp.where(avg_lane, prod, 0.0), axis=1, keepdims=True)
        zm = jnp.sum(jnp.where(avg_lane, 0.0, prod), axis=1, keepdims=True)
        gate = _bf(0.5 * jnp.tanh(_bf(_bf(za) + _bf(zm))) + 0.5)
        scale.append(jnp.broadcast_to(gate, (8, 128)))

    def store(idx, slot):
        return pltpu.make_async_copy(buf.at[idx], o_hbm.at[idx], sem_out.at[slot])

    for j in range(RAMP):
        for a in range(WA):
            p = (a + j) % NPH
            row = jnp.concatenate([scale[(8 * p + k) // WT] for k in range(8)], axis=1)
            buf[a, j] = (buf[a, j].astype(F32) * row).astype(BF16)
            if j == 0:
                store((a, j), j).start()
        if j > 0:
            store((pl.ds(0, WA), j), j).start()

    for u in range(NCG * WT):
        tab[u // 8, :, pl.ds(128 * (u % 8), 128)] = scale[u // WT]

    def block(i):
        return lax.shift_right_logical(i, 6) * WA, i & (NJ - 1)

    def write_body(lo, i, r):
        s0, j = block(i)
        for a in range(WA):
            p = jnp.where(r + a >= NPH, r + a - NPH, r + a)
            buf[s0 + a, j] = (buf[s0 + a, j].astype(F32) * tab[p]).astype(BF16)
        slot = WRING if lo >= NWRITE - WLAG else i & (WRING - 1)
        for k in range(8):
            store((pl.ds(s0, WA), j, slice(None), pl.ds(128 * k, 128)), slot).start()
        if lo >= WLAG:
            s1, j1 = block(i - WLAG)
            store((pl.ds(s1, WA), j1), (i - WLAG) & (WRING - 1)).wait()
        r = r + jnp.where(j == NJ - 1, (WA - (NJ - 1)) % NPH, 1)
        return jnp.where(r >= NPH, r - NPH, r)

    r = jnp.int32(RAMP)
    cuts = (RAMP, WLAG, NWRITE - WLAG, NWRITE)
    for lo, hi in zip(cuts[:-1], cuts[1:]):
        r = lax.fori_loop(lo, hi, functools.partial(write_body, lo), r)
    store((pl.ds(NSEG - WA, WA), pl.ds(NJ - WLAG, WLAG)), WRING).wait()


@jax.jit
def pallas_standalone__channel_attn_cbam__vision_kernel(
    x: jax.Array,
    w1: jax.Array,
    w2: jax.Array,
):
    assert x.shape == (1, H, W, C) and w1.shape == (C, R) and w2.shape == (R, C)
    out = pl.pallas_call(
        _cbam_kernel,
        out_shape=jax.ShapeDtypeStruct((NSEG, NJ, 8, CW), BF16),
        in_specs=[pl.BlockSpec(memory_space=pl.ANY)] * 3,
        out_specs=pl.BlockSpec(memory_space=pl.ANY),
        scratch_shapes=[
            pltpu.VMEM((NSEG, NJ, 8, CW), BF16),
            pltpu.VMEM((R, C), BF16),
            pltpu.VMEM((R, C), BF16),
            pltpu.VMEM((C, 128), F32),
            pltpu.VMEM((C, 128), F32),
            pltpu.VMEM((C, 128), F32),
            pltpu.VMEM((C, 128), F32),
            pltpu.VMEM((NPH, 8, CW), F32),
            pltpu.SemaphoreType.DMA((RING,)),
            pltpu.SemaphoreType.DMA((2,)),
            pltpu.SemaphoreType.DMA((WRING + 1,)),
        ],
        compiler_params=pltpu.CompilerParams(
            vmem_limit_bytes=64 * 1024 * 1024,
            disable_semaphore_checks=True,
            disable_bounds_checks=True,
        ),
    )(_to_view(x), w1.T, w2)
    return _from_view(out)
```
